```python
import os as _os
_os.environ.setdefault("JAX_PLATFORMS", "cpu")
import jax
import jax.numpy as jnp

def _softmax(x, axis=-1):
    return jax.nn.softmax(x, axis=axis)
def _gelu(x):
    return jax.nn.gelu(x, approximate=True)
def _silu(x):
    return jax.nn.silu(x)
def _sigmoid(x):
    return jax.nn.sigmoid(x)
def _layernorm(x, axis=-1, eps=1e-5):
    m = jnp.mean(x, axis=axis, keepdims=True)
    v = jnp.var(x, axis=axis, keepdims=True)
    return (x - m) / jnp.sqrt(v + eps)
def _scatter_add(tgt, idx, src, axis=0):
    return tgt.at[idx].add(src)
def _segment_sum(src, seg, n):
    return jax.ops.segment_sum(src, seg, n)
class _Rng:
    def __init__(self, key):
        self._k = key
    def _next(self):
        self._k, sub = jax.random.split(self._k)
        return sub
    def normal(self, shape):
        return jax.random.normal(self._next(), shape, dtype=jnp.bfloat16)
    def randint(self, lo, hi, shape):
        return jax.random.randint(self._next(), shape, lo, hi, dtype=jnp.int32)
    def uniform(self, shape, lo=0.0, hi=1.0):
        return jax.random.uniform(self._next(), shape, jnp.bfloat16, lo, hi)
    def permutation(self, n):
        return jax.random.permutation(self._next(), n)


kernel_name = 'standalone__gqa_softmax__near_ridge'

def setup_inputs():
    _rng = _Rng(jax.random.key(int.from_bytes(__import__("os").urandom(4), "little")))
    _w = (lambda a: (lambda t: t.astype(jnp.bfloat16) if jnp.issubdtype(t.dtype, jnp.floating) else t)(jnp.asarray(a)))
    B, Hq, Hkv, Sq, Sk, D = 8, 16, 8, 160, 2048, 256
    return {
        "q": _w((lambda *s: _rng.normal(s) * 0.05)(B, Hq, Sq, D)),
        "k": _w((lambda *s: _rng.normal(s) * 3.2)(B, Hkv, Sk, D)),
        "v": _w((lambda *s: _rng.normal(s) * 0.05)(B, Hkv, Sk, D)),
    }

def reference(q, k, v):
    B, Hq, Sq, D = q.shape
    Hkv = k.shape[1]
    rep = Hq // Hkv
    k = jnp.repeat(k, rep, axis=1)
    v = jnp.repeat(v, rep, axis=1)
    scale = D ** -0.5
    scores = jnp.einsum("bhqd,bhkd->bhqk", q, k) * scale
    p = _softmax(scores, axis=-1)
    return jnp.einsum("bhqk,bhkd->bhqd", p, v)
```

```python
import math

import jax
import jax.numpy as jnp
import jax.experimental.pallas as pl
import jax.experimental.pallas.tpu as pltpu

_NK = 8
_N = 2


@jax.jit
def pallas_standalone__gqa_softmax__near_ridge_kernel(
    q: jax.Array,
    k: jax.Array,
    v: jax.Array,
):
    B, Hq, Sq, D = q.shape
    Hkv, Sk = k.shape[1], k.shape[2]
    rep = Hq // Hkv
    M = rep * Sq
    U = B * Hkv
    n, nk = _N, _NK
    assert U % n == 0 and n % 2 == 0 and U >= 2 * n
    G = U // n
    kc = Sk // nk
    c2 = (D ** -0.5) * math.log2(math.e)
    q2 = q.reshape(U, M, D)
    k2 = k.reshape(U, Sk, D)
    v2 = v.reshape(U, Sk, D)

    def phase(q_ref, k_ref, v_ref, o_ref, p_ref, s_rd, m_rd, s_wr, m_wr,
              do_qk=True, do_pv=True):
        l = None
        m_new = None
        if do_pv:
            m_old = m_rd[...]
        if do_qk:
            qv = q_ref[...]
        for j in range(nk):
            sl = slice(j * kc, (j + 1) * kc)
            if do_pv:
                p = jnp.exp2((s_rd[:, sl] - m_old) * c2)
                lj = jnp.sum(p, axis=-1, keepdims=True)
                l = lj if l is None else l + lj
                p_ref[:, sl] = pltpu.bitcast(p.astype(jnp.bfloat16), jnp.uint32)
            if do_qk:
                s = jax.lax.dot_general(qv, k_ref[sl, :], (((1,), (1,)), ((), ())),
                                        preferred_element_type=jnp.float32)
                s_wr[:, sl] = s
                mj = jnp.max(s, axis=-1, keepdims=True)
                m_new = mj if m_new is None else jnp.maximum(m_new, mj)
        if do_pv:
            pb = pltpu.bitcast(p_ref[...], jnp.bfloat16)
            acc = jnp.dot(pb, v_ref[...], preferred_element_type=jnp.float32)
        if do_qk:
            m_wr[...] = m_new
        if do_pv:
            o_ref[...] = (acc / l).astype(o_ref.dtype)

    def kernel(q_hbm, k_hbm, v_hbm, o_hbm, qbuf, kbuf, vbuf, obuf,
               pa, pb, sa, ma, sb, mb, qsem, ksem, vsem, osem):
        g = pl.program_id(0)
        S = (sa, sb)
        Mx = (ma, mb)
        P = (pa, pb)

        def kq_start(gs):
            return jnp.minimum(n * (gs - 1) + 1, U - n)

        def q_cp(gs):
            return pltpu.make_async_copy(q_hbm.at[pl.ds(kq_start(gs), n)],
                                         qbuf.at[gs % 2], qsem.at[gs % 2])

        def k_cp(gs):
            return pltpu.make_async_copy(k_hbm.at[pl.ds(kq_start(gs), n)],
                                         kbuf.at[gs % 2], ksem.at[gs % 2])

        def v_cp(gs):
            return pltpu.make_async_copy(v_hbm.at[pl.ds(n * (gs - 1), n)],
                                         vbuf.at[gs % 2], vsem.at[gs % 2])

        def o_cp(gs):
            return pltpu.make_async_copy(obuf.at[gs % 2],
                                         o_hbm.at[pl.ds(n * (gs - 1), n)],
                                         osem.at[gs % 2])

        @pl.when(g == 0)
        def _():
            q0 = pltpu.make_async_copy(q_hbm.at[0], qbuf.at[0, 0], qsem.at[0])
            k0 = pltpu.make_async_copy(k_hbm.at[0], kbuf.at[0, 0], ksem.at[0])
            q0.start()
            k0.start()
            q_cp(1).start()
            k_cp(1).start()
            v_cp(1).start()
            q0.wait()
            k0.wait()
            phase(qbuf.at[0, 0], kbuf.at[0, 0], None, None, None, None, None,
                  sa, ma, do_pv=False)

        def main(last):
            slot = g % 2
            if not last:
                q_cp(g + 1).start()
                k_cp(g + 1).start()
                v_cp(g + 1).start()
            q_cp(g).wait()
            k_cp(g).wait()
            v_cp(g).wait()

            @pl.when(g >= 3)
            def _():
                o_cp(g - 2).wait()

            for t in range(n):
                do_qk = not (last and t == n - 1)
                tk = min(t + 1, n - 1) if last else t
                phase(qbuf.at[slot, tk], kbuf.at[slot, tk], vbuf.at[slot, t],
                      obuf.at[slot, t], P[t % 2], S[t % 2], Mx[t % 2],
                      S[(t + 1) % 2], Mx[(t + 1) % 2], do_qk=do_qk)
            o_cp(g).start()
            if last:
                o_cp(g - 1).wait()
                o_cp(g).wait()

        @pl.when(jnp.logical_and(g > 0, g < G))
        def _():
            main(False)

        @pl.when(g == G)
        def _():
            main(True)

    any_spec = pl.BlockSpec(memory_space=pl.ANY)
    out = pl.pallas_call(
        kernel,
        grid=(G + 1,),
        in_specs=[any_spec, any_spec, any_spec],
        out_specs=any_spec,
        out_shape=jax.ShapeDtypeStruct((U, M, D), q.dtype),
        scratch_shapes=[
            pltpu.VMEM((2, n, M, D), q.dtype),
            pltpu.VMEM((2, n, Sk, D), k.dtype),
            pltpu.VMEM((2, n, Sk, D), v.dtype),
            pltpu.VMEM((2, n, M, D), q.dtype),
            pltpu.VMEM((M // 2, Sk), jnp.uint32),
            pltpu.VMEM((M // 2, Sk), jnp.uint32),
            pltpu.VMEM((M, Sk), jnp.float32),
            pltpu.VMEM((M, 1), jnp.float32),
            pltpu.VMEM((M, Sk), jnp.float32),
            pltpu.VMEM((M, 1), jnp.float32),
            pltpu.SemaphoreType.DMA((2,)),
            pltpu.SemaphoreType.DMA((2,)),
            pltpu.SemaphoreType.DMA((2,)),
            pltpu.SemaphoreType.DMA((2,)),
        ],
        compiler_params=pltpu.CompilerParams(
            dimension_semantics=("arbitrary",),
            vmem_limit_bytes=100 * 1024 * 1024,
            disable_bounds_checks=True),
    )(q2, k2, v2)
    return out.reshape(B, Hq, Sq, D)
```

```python
import math

import jax
import jax.numpy as jnp
import jax.experimental.pallas as pl
import jax.experimental.pallas.tpu as pltpu

_NK = 8
_N = 2
_LAG = 2
_FINE = 5


@jax.jit
def pallas_standalone__gqa_softmax__near_ridge_kernel(
    q: jax.Array,
    k: jax.Array,
    v: jax.Array,
):
    B, Hq, Sq, D = q.shape
    Hkv, Sk = k.shape[1], k.shape[2]
    rep = Hq // Hkv
    M = rep * Sq
    U = B * Hkv
    n, nk, lag, F = _N, _NK, _LAG, _FINE
    G = U // n
    assert U % n == 0 and F + 2 <= G and Sk % (128 * nk) == 0 and M % 16 == 0
    kc = Sk // nk
    c2 = (D ** -0.5) * math.log2(math.e)
    q2 = q.reshape(U, M, D)
    k2 = k.reshape(U, Sk, D)
    v2 = v.reshape(U, Sk, D)

    def phase(q_ref, k_ref, v_ref, o_ref, p_ref, s_rd, m_rd, s_wr, m_wr,
              do_qk=True, do_pv=True, wait_kq=None, wait_v=None, v_late=False):
        if wait_kq is not None:
            wait_kq()
        if wait_v is not None and not v_late:
            wait_v()
        l = None
        m_new = None
        tok = {}
        if do_pv:
            m_old = m_rd[...]
        if do_qk:
            qv = q_ref[...]
        for j in range(nk):
            sl = slice(j * kc, (j + 1) * kc)
            if do_pv:
                if (j - lag) in tok:
                    t = tok[j - lag]
                    cj = jnp.where(t > jnp.inf, t, c2)
                else:
                    cj = c2
                p = jnp.exp2((s_rd[:, sl] - m_old) * cj)
                lj = jnp.sum(p, axis=-1, keepdims=True)
                l = lj if l is None else l + lj
                p_ref[:, sl] = pltpu.bitcast(p.astype(jnp.bfloat16), jnp.uint32)
            if do_qk:
                s = jax.lax.dot_general(qv, k_ref[sl, :], (((1,), (1,)), ((), ())),
                                        preferred_element_type=jnp.float32)
                s_wr[:, sl] = s
                tok[j] = s[0:1, :]
                mj = jnp.max(s, axis=-1, keepdims=True)
                m_new = mj if m_new is None else jnp.maximum(m_new, mj)
        if do_pv:
            if wait_v is not None and v_late:
                wait_v()
            pb = pltpu.bitcast(p_ref[...], jnp.bfloat16)
            acc = jnp.dot(pb, v_ref[...], preferred_element_type=jnp.float32)
        if do_qk:
            m_wr[...] = m_new
        if do_pv:
            o_ref[...] = (acc / l).astype(o_ref.dtype)

    def kernel(q_hbm, k_hbm, v_hbm, o_hbm, qbuf, kbuf, vbuf, obuf,
               pa, pb, sa, ma, sb, mb, usem, gsem, osem):
        g = pl.program_id(0)
        S = (sa, sb)
        Mx = (ma, mb)
        P = (pa, pb)

        def par(gs):
            return gs % 2 if isinstance(gs, int) else jnp.bitwise_and(gs, 1)

        def q_u(gs, t):
            return pltpu.make_async_copy(q_hbm.at[n * (gs - 1) + 1 + t],
                                         qbuf.at[par(gs), t], usem.at[par(gs), t])

        def k_u(gs, t):
            return pltpu.make_async_copy(k_hbm.at[n * (gs - 1) + 1 + t],
                                         kbuf.at[par(gs), t], usem.at[par(gs), n + t])

        def v_u(gs, t):
            return pltpu.make_async_copy(v_hbm.at[n * (gs - 1) + t],
                                         vbuf.at[par(gs), t], usem.at[par(gs), 2 * n + t])

        def kq_start(gs):
            return jnp.minimum(n * (gs - 1) + 1, U - n)

        def q_g(gs):
            return pltpu.make_async_copy(q_hbm.at[pl.ds(kq_start(gs), n)],
                                         qbuf.at[par(gs)], gsem.at[par(gs), 0])

        def k_g(gs):
            return pltpu.make_async_copy(k_hbm.at[pl.ds(kq_start(gs), n)],
                                         kbuf.at[par(gs)], gsem.at[par(gs), 1])

        def v_g(gs):
            return pltpu.make_async_copy(v_hbm.at[pl.ds(n * (gs - 1), n)],
                                         vbuf.at[par(gs)], gsem.at[par(gs), 2])

        def o_cp(gs):
            return pltpu.make_async_copy(obuf.at[par(gs)],
                                         o_hbm.at[pl.ds(n * (gs - 1), n)],
                                         osem.at[par(gs)])

        def prefetch_units(gs):
            for t in range(n):
                q_u(gs, t).start()
                k_u(gs, t).start()
                v_u(gs, t).start()

        def prefetch_group(gs):
            q_g(gs).start()
            k_g(gs).start()
            v_g(gs).start()

        def first():
            q_u(0, n - 1).start()
            k_u(0, n - 1).start()
            prefetch_units(1)
            q_u(0, n - 1).wait()
            k_u(0, n - 1).wait()
            phase(qbuf.at[0, n - 1], kbuf.at[0, n - 1], None, None, None, None, None,
                  sa, ma, do_pv=False)

        def main(kind, v_late=False):
            last = kind == "last"
            fine = kind == "fine"
            slot = par(g)

            if fine:
                @pl.when(g < F)
                def _():
                    prefetch_units(g + 1)

                @pl.when(g == F)
                def _():
                    prefetch_group(g + 1)

                @pl.when(g >= 3)
                def _():
                    o_cp(g - 2).wait()
            else:
                if not last:
                    prefetch_group(g + 1)
                q_g(g).wait()
                k_g(g).wait()
                v_g(g).wait()
                o_cp(g - 2).wait()

            def wait_kq(t):
                def f():
                    q_u(g, t).wait()
                    k_u(g, t).wait()
                return f

            def wait_v(t):
                return lambda: v_u(g, t).wait()

            for t in range(n):
                do_qk = not (last and t == n - 1)
                tk = min(t + 1, n - 1) if last else t
                phase(qbuf.at[slot, tk], kbuf.at[slot, tk], vbuf.at[slot, t],
                      obuf.at[slot, t], P[t % 2], S[t % 2], Mx[t % 2],
                      S[(t + 1) % 2], Mx[(t + 1) % 2], do_qk=do_qk,
                      wait_kq=wait_kq(t) if fine else None,
                      wait_v=wait_v(t) if fine else None, v_late=v_late)
            o_cp(g).start()
            if last:
                o_cp(g - 1).wait()
                o_cp(g).wait()

        def others():
            @pl.when(g == 0)
            def _():
                first()

            @pl.when(g == 1)
            def _():
                main("fine", v_late=True)

            @pl.when(jnp.logical_and(g > 1, g <= F))
            def _():
                main("fine")

            @pl.when(g == G)
            def _():
                main("last")

        jax.lax.cond(jnp.logical_and(g > F, g < G), lambda: main("coarse"), others)

    any_spec = pl.BlockSpec(memory_space=pl.ANY)
    out = pl.pallas_call(
        kernel,
        grid=(G + 1,),
        in_specs=[any_spec, any_spec, any_spec],
        out_specs=any_spec,
        out_shape=jax.ShapeDtypeStruct((U, M, D), q.dtype),
        scratch_shapes=[
            pltpu.VMEM((2, n, M, D), q.dtype),
            pltpu.VMEM((2, n, Sk, D), k.dtype),
            pltpu.VMEM((2, n, Sk, D), v.dtype),
            pltpu.VMEM((2, n, M, D), q.dtype),
            pltpu.VMEM((M // 2, Sk), jnp.uint32),
            pltpu.VMEM((M // 2, Sk), jnp.uint32),
            pltpu.VMEM((M, Sk), jnp.float32),
            pltpu.VMEM((M, 1), jnp.float32),
            pltpu.VMEM((M, Sk), jnp.float32),
            pltpu.VMEM((M, 1), jnp.float32),
            pltpu.SemaphoreType.DMA((2, 3 * n)),
            pltpu.SemaphoreType.DMA((2, 3)),
            pltpu.SemaphoreType.DMA((2,)),
        ],
        compiler_params=pltpu.CompilerParams(
            dimension_semantics=("arbitrary",),
            vmem_limit_bytes=100 * 1024 * 1024,
            disable_bounds_checks=True),
    )(q2, k2, v2)
    return out.reshape(B, Hq, Sq, D)
```

```python
import math

import jax
import jax.numpy as jnp
import jax.experimental.pallas as pl
import jax.experimental.pallas.tpu as pltpu

_NK = 8
_N = 2
_LAG = 2
_FINE = 5


@jax.jit
def pallas_standalone__gqa_softmax__near_ridge_kernel(
    q: jax.Array,
    k: jax.Array,
    v: jax.Array,
):
    B, Hq, Sq, D = q.shape
    Hkv, Sk = k.shape[1], k.shape[2]
    rep = Hq // Hkv
    M = rep * Sq
    U = B * Hkv
    n, nk, lag, F = _N, _NK, _LAG, _FINE
    G = U // n
    assert U % n == 0 and F + 2 <= G and Sk % (128 * nk) == 0 and M % 16 == 0
    kc = Sk // nk
    c2 = (D ** -0.5) * math.log2(math.e)
    q2 = q.reshape(U, M, D)
    k2 = k.reshape(U, Sk, D)
    v2 = v.reshape(U, Sk, D)

    def phase(q_ref, k_ref, v_ref, o_ref, p_ref, s_rd, m_rd, s_wr, m_wr,
              do_qk=True, do_pv=True, wait_kq=None, wait_v=None, v_late=False):
        if wait_kq is not None:
            wait_kq()
        if wait_v is not None and not v_late:
            wait_v()
        l = None
        m_new = None
        tok = {}
        if do_pv:
            m_old = m_rd[...]
        if do_qk:
            qv = q_ref[...]
        for j in range(nk):
            sl = slice(j * kc, (j + 1) * kc)
            if do_pv:
                if (j - lag) in tok:
                    t = tok[j - lag]
                    cj = jnp.where(t > jnp.inf, t, c2)
                else:
                    cj = c2
                p = jnp.exp2((s_rd[:, sl] - m_old) * cj)
                lj = jnp.sum(p, axis=-1, keepdims=True)
                l = lj if l is None else l + lj
                p_ref[:, sl] = pltpu.bitcast(p.astype(jnp.bfloat16), jnp.uint32)
            if do_qk:
                s = jax.lax.dot_general(qv, k_ref[sl, :], (((1,), (1,)), ((), ())),
                                        preferred_element_type=jnp.float32)
                s_wr[:, sl] = s
                tok[j] = s[0:1, :]
                mj = jnp.max(s, axis=-1, keepdims=True)
                m_new = mj if m_new is None else jnp.maximum(m_new, mj)
        if do_pv:
            if wait_v is not None and v_late:
                wait_v()
            pb = pltpu.bitcast(p_ref[...], jnp.bfloat16)
            acc = jnp.dot(pb, v_ref[...], preferred_element_type=jnp.float32)
        if do_qk:
            m_wr[...] = m_new
        if do_pv:
            o_ref[...] = (acc / l).astype(o_ref.dtype)

    def kernel(q_hbm, k_hbm, v_hbm, o_hbm, qbuf, kbuf, vbuf, obuf,
               pa, pb, sa, ma, sb, mb, usem, gsem, osem):
        g = pl.program_id(0)
        S = (sa, sb)
        Mx = (ma, mb)
        P = (pa, pb)

        def par(gs):
            return gs % 2 if isinstance(gs, int) else jnp.bitwise_and(gs, 1)

        def q_u(gs, t):
            return pltpu.make_async_copy(q_hbm.at[n * (gs - 1) + 1 + t],
                                         qbuf.at[par(gs), t], usem.at[par(gs), t])

        def k_u(gs, t):
            return pltpu.make_async_copy(k_hbm.at[n * (gs - 1) + 1 + t],
                                         kbuf.at[par(gs), t], usem.at[par(gs), n + t])

        def v_u(gs, t):
            return pltpu.make_async_copy(v_hbm.at[n * (gs - 1) + t],
                                         vbuf.at[par(gs), t], usem.at[par(gs), 2 * n + t])

        def kq_start(gs):
            return jnp.minimum(n * (gs - 1) + 1, U - n)

        def q_g(gs):
            return pltpu.make_async_copy(q_hbm.at[pl.ds(kq_start(gs), n)],
                                         qbuf.at[par(gs)], gsem.at[par(gs), 0])

        def k_g(gs):
            return pltpu.make_async_copy(k_hbm.at[pl.ds(kq_start(gs), n)],
                                         kbuf.at[par(gs)], gsem.at[par(gs), 1])

        def v_g(gs):
            return pltpu.make_async_copy(v_hbm.at[pl.ds(n * (gs - 1), n)],
                                         vbuf.at[par(gs)], gsem.at[par(gs), 2])

        def o_cp(gs):
            return pltpu.make_async_copy(obuf.at[par(gs)],
                                         o_hbm.at[pl.ds(n * (gs - 1), n)],
                                         osem.at[par(gs)])

        def prefetch_units(gs):
            for t in range(n):
                q_u(gs, t).start()
                k_u(gs, t).start()
                v_u(gs, t).start()

        def prefetch_group(gs):
            q_g(gs).start()
            k_g(gs).start()
            v_g(gs).start()

        def first():
            q_u(0, n - 1).start()
            k_u(0, n - 1).start()
            prefetch_units(1)
            q_u(0, n - 1).wait()
            k_u(0, n - 1).wait()
            phase(qbuf.at[0, n - 1], kbuf.at[0, n - 1], None, None, None, None, None,
                  sa, ma, do_pv=False)

        def main(kind, v_late=False):
            last = kind == "last"
            fine = kind == "fine"
            slot = par(g)

            if fine:
                @pl.when(g < F)
                def _():
                    prefetch_units(g + 1)

                @pl.when(g == F)
                def _():
                    prefetch_group(g + 1)

                @pl.when(g >= 3)
                def _():
                    o_cp(g - 2).wait()
            else:
                if not last:
                    prefetch_group(g + 1)
                q_g(g).wait()
                k_g(g).wait()
                v_g(g).wait()
                o_cp(g - 2).wait()

            def wait_kq(t):
                def f():
                    q_u(g, t).wait()
                    k_u(g, t).wait()
                return f

            def wait_v(t):
                return lambda: v_u(g, t).wait()

            def o_last(t):
                return pltpu.make_async_copy(obuf.at[slot, t], o_hbm.at[n * (g - 1) + t],
                                             usem.at[slot, t])

            for t in range(n):
                do_qk = not (last and t == n - 1)
                tk = min(t + 1, n - 1) if last else t
                phase(qbuf.at[slot, tk], kbuf.at[slot, tk], vbuf.at[slot, t],
                      obuf.at[slot, t], P[t % 2], S[t % 2], Mx[t % 2],
                      S[(t + 1) % 2], Mx[(t + 1) % 2], do_qk=do_qk,
                      wait_kq=wait_kq(t) if fine else None,
                      wait_v=wait_v(t) if fine else None, v_late=v_late)
                if last:
                    o_last(t).start()
            if last:
                o_cp(g - 1).wait()
                for t in range(n):
                    o_last(t).wait()
            else:
                o_cp(g).start()

        def others():
            @pl.when(g == 0)
            def _():
                first()

            @pl.when(g == 1)
            def _():
                main("fine", v_late=True)

            @pl.when(jnp.logical_and(g > 1, g <= F))
            def _():
                main("fine")

            @pl.when(g == G)
            def _():
                main("last")

        jax.lax.cond(jnp.logical_and(g > F, g < G), lambda: main("coarse"), others)

    any_spec = pl.BlockSpec(memory_space=pl.ANY)
    out = pl.pallas_call(
        kernel,
        grid=(G + 1,),
        in_specs=[any_spec, any_spec, any_spec],
        out_specs=any_spec,
        out_shape=jax.ShapeDtypeStruct((U, M, D), q.dtype),
        scratch_shapes=[
            pltpu.VMEM((2, n, M, D), q.dtype),
            pltpu.VMEM((2, n, Sk, D), k.dtype),
            pltpu.VMEM((2, n, Sk, D), v.dtype),
            pltpu.VMEM((2, n, M, D), q.dtype),
            pltpu.VMEM((M // 2, Sk), jnp.uint32),
            pltpu.VMEM((M // 2, Sk), jnp.uint32),
            pltpu.VMEM((M, Sk), jnp.float32),
            pltpu.VMEM((M, 1), jnp.float32),
            pltpu.VMEM((M, Sk), jnp.float32),
            pltpu.VMEM((M, 1), jnp.float32),
            pltpu.SemaphoreType.DMA((2, 3 * n)),
            pltpu.SemaphoreType.DMA((2, 3)),
            pltpu.SemaphoreType.DMA((2,)),
        ],
        compiler_params=pltpu.CompilerParams(
            dimension_semantics=("arbitrary",),
            vmem_limit_bytes=100 * 1024 * 1024,
            disable_bounds_checks=True),
    )(q2, k2, v2)
    return out.reshape(B, Hq, Sq, D)
```
